```python
import jax
import jax.numpy as jnp

def _softmax(x, axis=-1):
    return jax.nn.softmax(x, axis=axis)
def _gelu(x):
    return jax.nn.gelu(x, approximate=True)
def _silu(x):
    return jax.nn.silu(x)
def _sigmoid(x):
    return jax.nn.sigmoid(x)
def _layernorm(x, axis=-1, eps=1e-5):
    m = jnp.mean(x, axis=axis, keepdims=True)
    v = jnp.var(x, axis=axis, keepdims=True)
    return (x - m) / jnp.sqrt(v + eps)
def _scatter_add(tgt, idx, src, axis=0):
    return tgt.at[idx].add(src)
def _segment_sum(src, seg, n):
    return jax.ops.segment_sum(src, seg, n)
class _Rng:
    def __init__(self, key):
        self._k = key
    def _next(self):
        self._k, sub = jax.random.split(self._k)
        return sub
    def normal(self, shape):
        return jax.random.normal(self._next(), shape, dtype=jnp.bfloat16)
    def randint(self, lo, hi, shape):
        return jax.random.randint(self._next(), shape, lo, hi, dtype=jnp.int32)
    def uniform(self, shape, lo=0.0, hi=1.0):
        return jax.random.uniform(self._next(), shape, jnp.bfloat16, lo, hi)
    def permutation(self, n):
        return jax.random.permutation(self._next(), n)


kernel_name = 'concat_heads__ssm_conv_h3__compressed_kv_cla__prompt'

def setup_inputs():
    _rng = _Rng(jax.random.key(int.from_bytes(__import__("os").urandom(4), "little")))
    _w = (lambda a: (lambda t: t.astype(jnp.bfloat16) if jnp.issubdtype(t.dtype, jnp.floating) else t)(jnp.asarray(a)))
    def _A_setup():
        B, S, D = 1, 2048, 448
        ks = 4
        return {
            "q": _w((lambda *s: _rng.normal(s) * 0.05)(B, S, D)),
            "k": _w((lambda *s: _rng.normal(s) * 0.05)(B, S, D)),
            "v": _w((lambda *s: _rng.normal(s) * 0.05)(B, S, D)),
            "shift_k": _w((lambda *s: _rng.normal(s) * 0.05)(D, ks) * 0.5),
            "ssm_k": _w((lambda *s: _rng.normal(s) * 0.05)(D, S) * (1.0 / S ** 0.5)),
            "ssm_D": _w((lambda *s: _rng.normal(s) * 0.05)(D)),
        }
    _A_in = _A_setup()

    def _B_setup():
        B, H, Sq, Sk, D, M = 1, 16, 2048, 2048, 256, 448
        Dc = 4 * D
        return {
            "x": _w((lambda *s: _rng.normal(s) * 0.05)(B, Sq, M)),
            "c_kv": _w((lambda *s: _rng.normal(s) * 0.05)(B, Sk, Dc)),
            "w_q": _w((lambda *s: _rng.normal(s) * 0.05)(M, H, D) * (M ** -0.5)),
            "w_uk": _w((lambda *s: _rng.normal(s) * 0.05)(Dc, H, D) * (Dc ** -0.5)),
            "w_uv": _w((lambda *s: _rng.normal(s) * 0.05)(Dc, H, D) * (Dc ** -0.5)),
            "w_o": _w((lambda *s: _rng.normal(s) * 0.05)(H, D, M) * ((H * D) ** -0.5)),
        }
    _B_in = _B_setup()

    return {
        "A_q": _A_in["q"],
        "A_k": _A_in["k"],
        "A_v": _A_in["v"],
        "A_shift_k": _A_in["shift_k"],
        "A_ssm_k": _A_in["ssm_k"],
        "A_ssm_D": _A_in["ssm_D"],
        "B_x": _B_in["x"],
        "B_c_kv": _B_in["c_kv"],
        "B_w_q": _B_in["w_q"],
        "B_w_uk": _B_in["w_uk"],
        "B_w_uv": _B_in["w_uv"],
        "B_w_o": _B_in["w_o"],
    }

def reference(A_q, A_k, A_v, A_shift_k, A_ssm_k, A_ssm_D, B_x, B_c_kv, B_w_q, B_w_uk, B_w_uv, B_w_o):
    def _A_ref(q, k, v, shift_k, ssm_k, ssm_D):
        B, S, D = q.shape
        ks = shift_k.shape[-1]
        k_pad = jnp.pad(k, ((0, 0), (ks - 1, 0), (0, 0)))
        k_shift = jnp.zeros_like(k)
        for t in range(ks):
            k_shift = k_shift + k_pad[:, t:t + S, :] * shift_k[:, ks - 1 - t][None, None, :]
        kv = k_shift * v
        L = 2 * S
        kv_pad = jnp.pad(kv, ((0, 0), (0, S), (0, 0)))
        kf_pad = jnp.pad(ssm_k, ((0, 0), (0, S)))
        kv_f = (lambda x, axes=(-2,-1): jnp.fft.rfft2(x.astype(jnp.float32), axes=axes))(kv_pad[:, None, :, :], axes=(1, 2))
        kf_f = (lambda x, axes=(-2,-1): jnp.fft.rfft2(x.astype(jnp.float32), axes=axes))(kf_pad[:, None, :], axes=(1, 2))
        kf_f = (lambda x, *d: x.transpose(*d))(kf_f, 1, 2, 0)
        y_f = kv_f * kf_f[None, :, :, :]
        y = (lambda x, s, axes=(-2,-1): jnp.fft.irfft2(x, s=s, axes=axes).astype(jnp.bfloat16))(y_f, (1, L), axes=(1, 2))[:, 0, :S, :]
        y = y + kv * ssm_D[None, None, :]
        return q * y

    def _B_ref(x, c_kv, w_q, w_uk, w_uv, w_o):
        B, Sq, M = x.shape[0], x.shape[1], x.shape[2]
        Sk = c_kv.shape[1]
        H, D = w_q.shape[1], w_q.shape[2]
        q = jnp.einsum("bqm,mhd->bhqd", x, w_q)
        k = jnp.einsum("bkc,chd->bhkd", c_kv, w_uk)
        v = jnp.einsum("bkc,chd->bhkd", c_kv, w_uv)
        scores = jnp.einsum("bhqd,bhkd->bhqk", q, k) * (D ** -0.5)
        off = Sk - Sq
        qi = jnp.arange(Sq)[:, None]
        kj = jnp.arange(Sk)[None, :]
        cmask = kj <= (qi + off)
        scores = jnp.where(cmask[None, None], scores, -1e9)
        p = _softmax(scores, axis=-1)
        ctx = jnp.einsum("bhqk,bhkd->bhqd", p, v)
        return jnp.einsum("bhqd,hdm->bqm", ctx, w_o)

    a = _A_ref(A_q, A_k, A_v, A_shift_k, A_ssm_k, A_ssm_D)
    b = _B_ref(B_x, B_c_kv, B_w_q, B_w_uk, B_w_uv, B_w_o)
    return jnp.concatenate([a, b], axis=-1)
```

```python
import jax
import jax.numpy as jnp
import numpy as np
import jax.experimental.pallas as pl
import jax.experimental.pallas.tpu as pltpu

S, DA, KS = 2048, 448, 4
H, D, M, DC = 16, 256, 448, 1024
R = 64
G = R // 2 + 1
TS = 72
BQ = BK = 256
PM = 512
f32, bf16 = jnp.float32, jnp.bfloat16
NT = (((1,), (1,)), ((), ()))


def _dft_consts():
    n1, g, n2, k2 = np.arange(R // 2), np.arange(G), np.arange(R), np.arange(R)
    w = np.exp(-2j * np.pi * np.outer(g, n1) / R)
    f1 = np.stack([w.real, w.imag], 1).reshape(2 * G, R // 2)
    k = g[:, None, None] + R * k2[None, :, None]
    e = np.exp(-2j * np.pi * k * n2[None, None, :] / (R * R))
    f2 = np.block([[e.real, -e.imag], [e.imag, e.real]])
    ei = np.conj(e).transpose(0, 2, 1)
    f3 = np.block([[ei.real, -ei.imag], [ei.imag, ei.real]])
    cg = np.where((g == 0) | (g == R // 2), 1.0, 2.0) / (R * R)
    wi = np.conj(w) * cg[:, None]
    f4 = np.stack([wi.real, -wi.imag], 1).reshape(2 * G, R // 2).T
    cast = lambda a: np.asarray(a, np.float32).astype(bf16)
    return cast(f1), cast(f2), cast(f3), cast(f4), cast(np.eye(128))


def _dot(a, b):
    return jnp.dot(a, b, preferred_element_type=f32)


def _dot_nt(a, b):
    return jax.lax.dot_general(a, b, NT, preferred_element_type=f32)


def _branch_a(aq, ak, av, sk, ssk, sd, f1, f2, f3, f4, eye, kp, u, kt, t1u, t1k, o_ref):
    tiles = [(c, slice(c * 128, min((c + 1) * 128, DA)), min(128, DA - c * 128)) for c in range(4)]
    taps = sk[...].astype(f32)
    tr = lambda ref, j: _dot_nt(eye[...], ref[:, j * 128:(j + 1) * 128])
    kp[0:8, :] = jnp.zeros((8, DA), f32)
    for j in range(S // 128):
        kp[8 + j * 128:8 + (j + 1) * 128, :] = tr(ak, j)
    for c in (u, kt):
        c[3, :, 64:] = jnp.zeros((S, 64), f32)
    for i in range(S // 256):
        r0 = i * 256
        ks = sum(kp[8 + r0 - t:8 + r0 - t + 256, :] * taps[t:t + 1, :] for t in range(KS))
        kv = (ks.astype(bf16).astype(f32) * jnp.concatenate([tr(av, 2 * i), tr(av, 2 * i + 1)], 0)).astype(bf16).astype(f32)
        for c, ls, n in tiles:
            u[c, r0:r0 + 256, :n] = kv[:, ls]
    for j in range(S // 128):
        kk = tr(ssk, j)
        for c, ls, n in tiles:
            kt[c, j * 128:(j + 1) * 128, :n] = kk[:, ls]
    for src, dst in ((u, t1u), (kt, t1k)):
        for n2 in range(R):
            rhs = jnp.concatenate([src[c, pl.ds(n2, R // 2, stride=R), :] for c in range(4)], 1)
            out = _dot(f1[...], rhs.astype(bf16))
            for c in range(4):
                dst[c, n2 * TS:n2 * TS + 2 * G, :] = out[:, c * 128:(c + 1) * 128]
    for g in range(G):
        def spec(t):
            rhs = jnp.concatenate([
                jnp.concatenate([t[c, pl.ds(2 * g + ri, R, stride=TS), :] for c in range(4)], 1)
                for ri in range(2)], 0)
            z = _dot(f2[g], rhs.astype(bf16))
            return z[:R], z[R:]
        ur, ui = spec(t1u)
        kr, ki = spec(t1k)
        y = jnp.concatenate([ur * kr - ui * ki, ur * ki + ui * kr], 0).astype(bf16)
        z = _dot(f3[g], y)
        for c in range(4):
            for ri in range(2):
                t1u[c, pl.ds(2 * g + ri, R, stride=TS), :] = z[ri * R:(ri + 1) * R, c * 128:(c + 1) * 128]
    for n2 in range(R):
        rhs = jnp.concatenate([t1u[c, n2 * TS:n2 * TS + 2 * G, :] for c in range(4)], 1)
        out = _dot(f4[...], rhs.astype(bf16))
        for c in range(4):
            kt[c, pl.ds(n2, R // 2, stride=R), :] = out[:, c * 128:(c + 1) * 128]
    dd = sd[...].astype(f32)
    for i in range(S // 128):
        rs = slice(i * 128, (i + 1) * 128)
        qq = tr(aq, i)
        for c, ls, n in tiles:
            y = kt[c, rs, :n] + u[c, rs, :n] * dd[:, ls]
            o_ref[rs, ls] = (qq[:, ls] * y).astype(bf16)


def _kernel(aq, ak, av, sk, ssk, sd, f1, f2, f3, f4, eye, xt_ref, c_ref, wq_h, wk_h, wv_h, wo_ref,
            o_ref, kp, u, kt, t1u, t1k, wq0, wq1, wk0, wk1, wv0, wv1, pq, pk, pv,
            wq_s, wk_s, wv_s, x_ref, q_s, k_s, v_s, acc, sem):
    h = pl.program_id(0)
    raw = ((wq_h, (wq0, wq1), pq, M), (wk_h, (wk0, wk1), pk, DC), (wv_h, (wv0, wv1), pv, DC))

    @pl.when(h == 0)
    def _():
        cps = [pltpu.make_async_copy(w.at[:, pl.ds(c * 128, 128)], bufs[c], sem.at[2 * i + c])
               for i, (w, bufs, _, _) in enumerate(raw) for c in range(2)]
        for cp in cps:
            cp.start()
        _branch_a(aq, ak, av, sk, ssk, sd, f1, f2, f3, f4, eye, kp, u, kt, t1u, t1k, o_ref)
        acc[...] = jnp.zeros_like(acc)
        for j in range(S // 128):
            x_ref[j * 128:(j + 1) * 128, :] = _dot_nt(eye[...], xt_ref[:, j * 128:(j + 1) * 128]).astype(bf16)
        for cp in cps:
            cp.wait()

    for j in range(H // 2):
        @pl.when(h == 2 * j)
        def _(j=j):
            for _, bufs, pair, rows in raw:
                for c in range(2):
                    pair[:, c * 128:(c + 1) * 128] = bufs[c].bitcast(jnp.uint32)[pl.ds(j, rows, stride=H // 2), :]

    sh = ((1 - (h & 1)) * 16).astype(jnp.uint32)
    for pair, w_s in ((pq, wq_s), (pk, wk_s), (pv, wv_s)):
        w_s[...] = pltpu.bitcast((pair[...] << sh) & jnp.uint32(0xFFFF0000), f32).astype(bf16)

    sc = np.float32(np.log2(np.e) * D ** -0.5)
    for i in range(S // PM):
        r = slice(i * PM, (i + 1) * PM)
        q_s[r, :] = (_dot(x_ref[r, :], wq_s[...]) * sc).astype(bf16)
        k_s[r, :] = _dot(c_ref[r, :], wk_s[...]).astype(bf16)
        v_s[r, :] = _dot(c_ref[r, :], wv_s[...]).astype(bf16)
    for i in range(S // BQ):
        r = slice(i * BQ, (i + 1) * BQ)
        q = q_s[r, :]
        ss = []
        for j in range(i + 1):
            s = _dot_nt(q, k_s[j * BK:(j + 1) * BK, :])
            if j == i:
                ri = jax.lax.broadcasted_iota(jnp.int32, (BQ, BK), 0)
                ci = jax.lax.broadcasted_iota(jnp.int32, (BQ, BK), 1)
                s = jnp.where(ci <= ri, s, -1e9)
            m = s if j == 0 else jnp.maximum(m, s)
            ss.append(s)
        m = jnp.max(m, axis=1, keepdims=True)
        for j in range(i + 1):
            p = jnp.exp2(ss[j] - m)
            l = p if j == 0 else l + p
            pv_ = _dot(p.astype(bf16), v_s[j * BK:(j + 1) * BK, :])
            o = pv_ if j == 0 else o + pv_
        ctx = (o * (1.0 / jnp.sum(l, axis=1, keepdims=True))).astype(bf16)
        acc[64:, r] += _dot_nt(wo_ref[...], ctx)

    @pl.when(h == H - 1)
    def _():
        lane = jax.lax.broadcasted_iota(jnp.int32, (128, 128), 1)
        for j in range(S // 128):
            rs = slice(j * 128, (j + 1) * 128)
            b = _dot_nt(eye[...], acc[:, rs].astype(bf16)).astype(bf16)
            o_ref[rs, 384:512] = jnp.where(lane < 64, o_ref[rs, 384:512], b[:, :128])
            o_ref[rs, 512:] = b[:, 128:]


@jax.jit
def pallas_concat_heads__ssm_conv_h3__compressed_kv_cla__prompt_kernel(
    A_q, A_k, A_v, A_shift_k, A_ssm_k, A_ssm_D, B_x, B_c_kv, B_w_q, B_w_uk, B_w_uv, B_w_o,
):
    consts = _dft_consts()
    vm = [A_q[0].T, A_k[0].T, A_v[0].T, A_shift_k.T, A_ssm_k, A_ssm_D[None], *consts, B_x[0].T, B_c_kv[0]]
    hbm = [B_w_q.reshape(M * H, D), B_w_uk.reshape(DC * H, D), B_w_uv.reshape(DC * H, D)]
    whole = lambda a: pl.BlockSpec(a.shape, lambda h, n=a.ndim: (0,) * n, pipeline_mode=pl.Buffered(1))
    V = pltpu.VMEM
    out = pl.pallas_call(
        _kernel,
        grid=(H,),
        in_specs=[whole(a) for a in vm] + [pl.BlockSpec(memory_space=pl.ANY)] * 3
        + [pl.BlockSpec((M, D), lambda h: (h, 0))],
        out_specs=pl.BlockSpec((S, 2 * M), lambda h: (0, 0)),
        out_shape=jax.ShapeDtypeStruct((S, DA + M), bf16),
        scratch_shapes=[V((S + 8, DA), f32), V((4, S, 128), f32), V((4, S, 128), f32),
                        V((4, R * TS, 128), f32), V((4, R * TS, 128), f32)]
        + [V((M * H, 128), bf16)] * 2 + [V((DC * H, 128), bf16)] * 4
        + [V((M, D), jnp.uint32), V((DC, D), jnp.uint32), V((DC, D), jnp.uint32)]
        + [V((M, D), bf16), V((DC, D), bf16), V((DC, D), bf16), V((S, M), bf16)]
        + [V((S, D), bf16)] * 3 + [V((512, S), f32), pltpu.SemaphoreType.DMA((6,))],
        compiler_params=pltpu.CompilerParams(
            dimension_semantics=("arbitrary",), vmem_limit_bytes=120 << 20),
        name="h3_cla",
    )(*vm, *hbm, B_w_o.transpose(0, 2, 1).reshape(H * M, D))
    return out[None]
```

```python
import jax
import jax.numpy as jnp
import numpy as np
import jax.experimental.pallas as pl
import jax.experimental.pallas.tpu as pltpu

S, DA, KS = 2048, 448, 4
H, D, M, DC = 16, 256, 448, 1024
R = 64
G = R // 2 + 1
TS = 72
BQ = BK = 256
PM = 1024
f32, bf16 = jnp.float32, jnp.bfloat16
NT = (((1,), (1,)), ((), ()))


def _dft_consts():
    n1, g, n2, k2 = np.arange(R // 2), np.arange(G), np.arange(R), np.arange(R)
    w = np.exp(-2j * np.pi * np.outer(g, n1) / R)
    f1 = np.stack([w.real, w.imag], 1).reshape(2 * G, R // 2)
    k = g[:, None, None] + R * k2[None, :, None]
    e = np.exp(-2j * np.pi * k * n2[None, None, :] / (R * R))
    f2 = np.block([[e.real, -e.imag], [e.imag, e.real]])
    ei = np.conj(e).transpose(0, 2, 1)
    f3 = np.block([[ei.real, -ei.imag], [ei.imag, ei.real]])
    cg = np.where((g == 0) | (g == R // 2), 1.0, 2.0) / (R * R)
    wi = np.conj(w) * cg[:, None]
    f4 = np.stack([wi.real, -wi.imag], 1).reshape(2 * G, R // 2).T
    cast = lambda a: np.asarray(a, np.float32).astype(bf16)
    return cast(f1), cast(f2), cast(f3), cast(f4), cast(np.eye(128))


def _dot(a, b):
    return jnp.dot(a, b, preferred_element_type=f32)


def _dot_nt(a, b):
    return jax.lax.dot_general(a, b, NT, preferred_element_type=f32)


def _tr(eye, ref, j):
    return _dot_nt(eye[...], ref[:, pl.ds(pl.multiple_of(j * 128, 128), 128)].astype(bf16))


def _branch_a(aq, ak, av, sk, ssk, sd, f1, f2, f3, f4, eye, kp, u, kt, t1u, t1k, o_ref, fcopies):
    tiles = [(c, slice(c * 128, min((c + 1) * 128, DA)), min(128, DA - c * 128)) for c in range(4)]
    taps = sk[...].astype(f32)
    dd = sd[...].astype(f32)
    kp[0:8, :] = jnp.zeros((8, DA), f32)
    for c in (u, kt):
        c[3, :, 64:] = jnp.zeros((R // 2 * TS, 64), f32)

    def chunks(j):
        return [(slice(e * R, (e + 1) * R), pl.ds(pl.multiple_of((2 * j + e) * TS, 8), R)) for e in range(2)]

    @pl.loop(0, S // 128)
    def _(j):
        r0 = pl.multiple_of(j * 128, 128)
        kp[pl.ds(8 + r0, 128), :] = _tr(eye, ak, j)
        kw = kp[pl.ds(r0, 136), :]
        ks = sum(kw[8 - t:136 - t] * taps[t:t + 1, :] for t in range(KS))
        kv = (ks.astype(bf16).astype(f32) * _tr(eye, av, j)).astype(bf16).astype(f32)
        kk = _tr(eye, ssk, j)
        for src, dst in chunks(j):
            for c, ls, n in tiles:
                u[c, dst, :n] = kv[src, ls]
                kt[c, dst, :n] = kk[src, ls]

    for src, dst in ((u, t1u), (kt, t1k)):
        for n2 in range(R):
            rhs = jnp.concatenate([src[c, pl.ds(n2, R // 2, stride=TS), :] for c in range(4)], 1)
            out = _dot(f1[...], rhs.astype(bf16))
            for c in range(4):
                dst[c, pl.ds(n2, 2 * G, stride=TS), :] = out[:, c * 128:(c + 1) * 128]

    for cp in fcopies:
        cp.wait()

    @pl.loop(0, G)
    def _(g):
        rows = [pl.ds(pl.multiple_of((2 * g + ri) * TS, 8), R) for ri in range(2)]

        def spec(t):
            rhs = jnp.concatenate([jnp.concatenate([t[c, r, :] for c in range(4)], 1) for r in rows], 0)
            z = _dot(f2[g], rhs.astype(bf16))
            return z[:R], z[R:]
        ur, ui = spec(t1u)
        kr, ki = spec(t1k)
        y = jnp.concatenate([ur * kr - ui * ki, ur * ki + ui * kr], 0).astype(bf16)
        z = _dot(f3[g], y)
        for c in range(4):
            for ri in range(2):
                t1u[c, rows[ri], :] = z[ri * R:(ri + 1) * R, c * 128:(c + 1) * 128]

    for n2 in range(R):
        rhs = jnp.concatenate([t1u[c, pl.ds(n2, 2 * G, stride=TS), :] for c in range(4)], 1)
        out = _dot(f4[...], rhs.astype(bf16))
        for c in range(4):
            kt[c, pl.ds(n2, R // 2, stride=TS), :] = out[:, c * 128:(c + 1) * 128]

    @pl.loop(0, S // 128)
    def _(j):
        qq = _tr(eye, aq, j)
        for e, (src, dst) in enumerate(chunks(j)):
            for c, ls, n in tiles:
                y = kt[c, dst, :n] + u[c, dst, :n] * dd[:, ls]
                o_ref[pl.ds(pl.multiple_of(j * 128 + e * R, R), R), ls] = (qq[src, ls] * y).astype(bf16)


def _kernel(aq, ak, av, sk, ssk, sd, f1, f4, eye, xt_h, c_h, f2_h, f3_h, wq_h, wk_h, wv_h, wo_ref,
            o_ref, kp, u, kt, t1u, t1k, wq0, wq1, wk0, wk1, wv0, wv1, pq, pk, pv,
            wq_s, wk_s, wv_s, x_ref, q_s, k_s, v_s, acc, sem, xt_ref, c_ref, f2, f3):
    h = pl.program_id(0)
    raw = ((wq_h, (wq0, wq1), pq, M), (wk_h, (wk0, wk1), pk, DC), (wv_h, (wv0, wv1), pv, DC))

    @pl.when(h == 0)
    def _():
        cps = [pltpu.make_async_copy(w.at[:, pl.ds(c * 128, 128)], bufs[c], sem.at[2 * i + c])
               for i, (w, bufs, _, _) in enumerate(raw) for c in range(2)]
        cps = [pltpu.make_async_copy(a, b, sem.at[6 + i]) for i, (a, b) in enumerate(
            ((f2_h, f2), (f3_h, f3), (xt_h, xt_ref), (c_h, c_ref)))] + cps
        for cp in cps:
            cp.start()
        _branch_a(aq, ak, av, sk, ssk, sd, f1, f2, f3, f4, eye, kp, u, kt, t1u, t1k, o_ref, cps[:2])
        cps[2].wait()
        acc[...] = jnp.zeros_like(acc)

        @pl.loop(0, S // 128)
        def _(j):
            x_ref[pl.ds(pl.multiple_of(j * 128, 128), 128), :] = _tr(eye, xt_ref, j).astype(bf16)
        for cp in cps[3:]:
            cp.wait()

    for j in range(H // 2):
        @pl.when(h == 2 * j)
        def _(j=j):
            for _, bufs, pair, rows in raw:
                for c in range(2):
                    pair[:, c * 128:(c + 1) * 128] = bufs[c].bitcast(jnp.uint32)[pl.ds(j, rows, stride=H // 2), :]

    sh = ((1 - (h & 1)) * 16).astype(jnp.uint32)
    for pair, w_s in ((pq, wq_s), (pk, wk_s), (pv, wv_s)):
        w_s[...] = pltpu.bitcast((pair[...] << sh) & jnp.uint32(0xFFFF0000), f32).astype(bf16)

    sc = np.float32(np.log2(np.e) * D ** -0.5)

    @pl.loop(0, S // PM)
    def _(i):
        r = pl.ds(pl.multiple_of(i * PM, PM), PM)
        q_s[r, :] = (_dot(x_ref[r, :], wq_s[...]) * sc).astype(bf16)
        k_s[r, :] = _dot(c_ref[r, :], wk_s[...]).astype(bf16)
        v_s[r, :] = _dot(c_ref[r, :], wv_s[...]).astype(bf16)
    for i in range(S // BQ):
        r = slice(i * BQ, (i + 1) * BQ)
        q = q_s[r, :]
        hb = BQ // 2
        ka, kb = slice(i * BQ, i * BQ + hb), slice(i * BQ + hb, (i + 1) * BQ)
        causal = lambda s: jnp.where(jax.lax.broadcasted_iota(jnp.int32, s.shape, 1)
                                     <= jax.lax.broadcasted_iota(jnp.int32, s.shape, 0), s, -1e9)
        sa = causal(_dot_nt(q, k_s[ka, :]))
        sb = causal(_dot_nt(q[hb:], k_s[kb, :]))
        m = jnp.concatenate([sa[:hb], jnp.maximum(sa[hb:], sb)], 0)
        ss = [_dot_nt(q, k_s[j * BK:(j + 1) * BK, :]) for j in range(i)]
        for s in ss:
            m = jnp.maximum(m, jnp.maximum(s[:, :hb], s[:, hb:]))
        m = jnp.max(m, axis=1, keepdims=True)
        pa, pb = jnp.exp2(sa - m), jnp.exp2(sb - m[hb:])
        l = jnp.concatenate([pa[:hb], pa[hb:] + pb], 0)
        o = _dot(pa.astype(bf16), v_s[ka, :])
        o = jnp.concatenate([o[:hb], o[hb:] + _dot(pb.astype(bf16), v_s[kb, :])], 0)
        for j, s in enumerate(ss):
            p = jnp.exp2(s - m)
            l = l + (p[:, :hb] + p[:, hb:])
            o = o + _dot(p.astype(bf16), v_s[j * BK:(j + 1) * BK, :])
        ctx = (o * (1.0 / jnp.sum(l, axis=1, keepdims=True))).astype(bf16)
        acc[64:, r] += _dot_nt(wo_ref[...], ctx)

    @pl.when(h == H - 1)
    def _():
        lane = jax.lax.broadcasted_iota(jnp.int32, (128, 128), 1)

        @pl.loop(0, S // 128)
        def _(j):
            rs = pl.ds(pl.multiple_of(j * 128, 128), 128)
            b = _tr(eye, acc, j).astype(bf16)
            o_ref[rs, 384:512] = jnp.where(lane < 64, o_ref[rs, 384:512], b[:, :128])
            o_ref[rs, 512:] = b[:, 128:]


@jax.jit
def pallas_concat_heads__ssm_conv_h3__compressed_kv_cla__prompt_kernel(
    A_q, A_k, A_v, A_shift_k, A_ssm_k, A_ssm_D, B_x, B_c_kv, B_w_q, B_w_uk, B_w_uv, B_w_o,
):
    f1, f2, f3, f4, eye = _dft_consts()
    vm = [A_q[0].T, A_k[0].T, A_v[0].T, A_shift_k.T, A_ssm_k, A_ssm_D[None], f1, f4, eye]
    hbm = [B_x[0].T, B_c_kv[0], f2, f3, B_w_q.reshape(M * H, D), B_w_uk.reshape(DC * H, D), B_w_uv.reshape(DC * H, D)]
    whole = lambda a: pl.BlockSpec(a.shape, lambda h, n=a.ndim: (0,) * n, pipeline_mode=pl.Buffered(1))
    V = pltpu.VMEM
    out = pl.pallas_call(
        _kernel,
        grid=(H,),
        in_specs=[whole(a) for a in vm] + [pl.BlockSpec(memory_space=pl.ANY)] * 7
        + [pl.BlockSpec((M, D), lambda h: (h, 0))],
        out_specs=pl.BlockSpec((S, 2 * M), lambda h: (0, 0)),
        out_shape=jax.ShapeDtypeStruct((S, DA + M), bf16),
        scratch_shapes=[V((S + 8, DA), f32), V((4, R // 2 * TS, 128), f32), V((4, R // 2 * TS, 128), f32),
                        V((4, 2 * G * TS, 128), f32), V((4, 2 * G * TS, 128), f32)]
        + [V((M * H, 128), bf16)] * 2 + [V((DC * H, 128), bf16)] * 4
        + [V((M, D), jnp.uint32), V((DC, D), jnp.uint32), V((DC, D), jnp.uint32)]
        + [V((M, D), bf16), V((DC, D), bf16), V((DC, D), bf16), V((S, M), bf16)]
        + [V((S, D), bf16)] * 3 + [V((512, S), f32), pltpu.SemaphoreType.DMA((10,))]
        + [V(a.shape, bf16) for a in hbm[:4]],
        compiler_params=pltpu.CompilerParams(
            dimension_semantics=("arbitrary",), vmem_limit_bytes=120 << 20),
        name="h3_cla",
    )(*vm, *hbm, B_w_o.transpose(0, 2, 1).reshape(H * M, D))
    return out[None]
```
